```python
import os as _os
_os.environ.setdefault("JAX_PLATFORMS", "cpu")
import jax
import jax.numpy as jnp

def _softmax(x, axis=-1):
    return jax.nn.softmax(x, axis=axis)
def _gelu(x):
    return jax.nn.gelu(x, approximate=True)
def _silu(x):
    return jax.nn.silu(x)
def _sigmoid(x):
    return jax.nn.sigmoid(x)
def _layernorm(x, axis=-1, eps=1e-5):
    m = jnp.mean(x, axis=axis, keepdims=True)
    v = jnp.var(x, axis=axis, keepdims=True)
    return (x - m) / jnp.sqrt(v + eps)
def _scatter_add(tgt, idx, src, axis=0):
    return tgt.at[idx].add(src)
def _segment_sum(src, seg, n):
    return jax.ops.segment_sum(src, seg, n)
class _Rng:
    def __init__(self, key):
        self._k = key
    def _next(self):
        self._k, sub = jax.random.split(self._k)
        return sub
    def normal(self, shape):
        return jax.random.normal(self._next(), shape, dtype=jnp.bfloat16)
    def randint(self, lo, hi, shape):
        return jax.random.randint(self._next(), shape, lo, hi, dtype=jnp.int32)
    def uniform(self, shape, lo=0.0, hi=1.0):
        return jax.random.uniform(self._next(), shape, jnp.bfloat16, lo, hi)
    def permutation(self, n):
        return jax.random.permutation(self._next(), n)


kernel_name = 'standalone__gqa_softmax__decode'

def setup_inputs():
    _rng = _Rng(jax.random.key(int.from_bytes(__import__("os").urandom(4), "little")))
    _w = (lambda a: (lambda t: t.astype(jnp.bfloat16) if jnp.issubdtype(t.dtype, jnp.floating) else t)(jnp.asarray(a)))
    B, Hq, Hkv, Sq, Sk, D = 8, 32, 32, 1, 4096, 128
    return {
        "q": _w((lambda *s: _rng.normal(s) * 0.4)(B, Hq, Sq, D)),
        "k": _w((lambda *s: _rng.normal(s) * 0.4)(B, Hkv, Sk, D)),
        "v": _w((lambda *s: _rng.normal(s) * 0.05)(B, Hkv, Sk, D)),
    }

def reference(q, k, v):
    B, Hq, Sq, D = q.shape
    Hkv = k.shape[1]
    rep = Hq // Hkv
    k = jnp.repeat(k, rep, axis=1)
    v = jnp.repeat(v, rep, axis=1)
    scale = D ** -0.5
    scores = jnp.einsum("bhqd,bhkd->bhqk", q, k) * scale
    p = _softmax(scores, axis=-1)
    return jnp.einsum("bhqk,bhkd->bhqd", p, v)
```

```python
import jax
import jax.numpy as jnp
import jax.experimental.pallas as pl
import jax.experimental.pallas.tpu as pltpu

_ROWS = 128
_QGROUP = 2
_QPHASE = 1
_NSLOTS = 4
_INFLIGHT = 3


@jax.jit
def pallas_standalone__gqa_softmax__decode_kernel(
    q: jax.Array,
    k: jax.Array,
    v: jax.Array,
):
    B, Hq, Sq, D = q.shape
    Hkv, Sk = k.shape[1], k.shape[2]
    G = (Hq // Hkv) * Sq
    N = B * Hkv
    rows = _ROWS if Sk % _ROWS == 0 else Sk
    nch = Sk // rows
    scale = D ** -0.5

    q2 = q.reshape(N * G, D)
    k3 = k.reshape(N, Sk, D)
    v3 = v.reshape(N, Sk, D)

    def kernel_function(q_hbm, k_hbm, v_hbm, o_ref, kb, vb, qb, qf, of, sems, qsem):
        def start(head, slot):
            for c in range(nch):
                o = c * rows
                prio = ((c + _QPHASE) // _QGROUP) % 2
                pltpu.make_async_copy(
                    k_hbm.at[head, pl.ds(o, rows)], kb.at[slot, pl.ds(o, rows)],
                    sems.at[0, slot]).start(priority=prio)
                pltpu.make_async_copy(
                    v_hbm.at[head, pl.ds(o, rows)], vb.at[slot, pl.ds(o, rows)],
                    sems.at[1, slot]).start(priority=1 - prio)

        def wait(slot):
            pltpu.make_async_copy(kb.at[slot], kb.at[slot], sems.at[0, slot]).wait()
            pltpu.make_async_copy(vb.at[slot], vb.at[slot], sems.at[1, slot]).wait()

        q_copy = pltpu.make_async_copy(q_hbm, qb, qsem)
        q_copy.start()
        for j in range(min(_INFLIGHT, N)):
            start(j, j)
        q_copy.wait()
        qf[...] = qb[...].astype(jnp.float32)

        def body(h, carry):
            slot = jax.lax.rem(h, _NSLOTS)
            wait(slot)

            @pl.when(h + _INFLIGHT < N)
            def _():
                start(h + _INFLIGHT, jax.lax.rem(h + _INFLIGHT, _NSLOTS))

            qh = qf[pl.ds(h * G, G), :].astype(jnp.bfloat16)
            s = jax.lax.dot_general(
                qh, kb[slot], (((1,), (1,)), ((), ())),
                preferred_element_type=jnp.float32) * scale
            m = jnp.max(s, axis=-1, keepdims=True)
            p = jnp.exp(s - m)
            l = jnp.sum(p, axis=-1, keepdims=True)
            o = jnp.dot(p.astype(jnp.bfloat16), vb[slot],
                        preferred_element_type=jnp.float32)
            of[pl.ds(h * G, G), :] = o / l
            return carry

        jax.lax.fori_loop(0, N, body, 0)
        o_ref[...] = of[...].astype(o_ref.dtype)

    out = pl.pallas_call(
        kernel_function,
        in_specs=[pl.BlockSpec(memory_space=pl.ANY)] * 3,
        out_specs=pl.BlockSpec(memory_space=pltpu.VMEM),
        out_shape=jax.ShapeDtypeStruct((N * G, D), q.dtype),
        scratch_shapes=[
            pltpu.VMEM((_NSLOTS, Sk, D), k.dtype),
            pltpu.VMEM((_NSLOTS, Sk, D), v.dtype),
            pltpu.VMEM((N * G, D), q.dtype),
            pltpu.VMEM((N * G, D), jnp.float32),
            pltpu.VMEM((N * G, D), jnp.float32),
            pltpu.SemaphoreType.DMA((2, _NSLOTS)),
            pltpu.SemaphoreType.DMA(()),
        ],
        compiler_params=pltpu.CompilerParams(vmem_limit_bytes=64 * 1024 * 1024),
    )(q2, k3, v3)
    return out.reshape(B, Hq, Sq, D)
```

```python
import jax
import jax.numpy as jnp
import jax.experimental.pallas as pl
import jax.experimental.pallas.tpu as pltpu

_ROWS = 128
_QGROUP = 2
_QPHASE = 1
_NSLOTS = 4
_INFLIGHT = 3


@jax.jit
def pallas_standalone__gqa_softmax__decode_kernel(
    q: jax.Array,
    k: jax.Array,
    v: jax.Array,
):
    B, Hq, Sq, D = q.shape
    Hkv, Sk = k.shape[1], k.shape[2]
    G = (Hq // Hkv) * Sq
    N = B * Hkv
    assert N > _INFLIGHT
    rows = _ROWS if Sk % _ROWS == 0 else Sk
    nch = Sk // rows
    scale = D ** -0.5

    q2 = q.reshape(N * G, D)
    k3 = k.reshape(N, Sk, D)
    v3 = v.reshape(N, Sk, D)

    def prio(c):
        return ((c + _QPHASE) // _QGROUP) % 2

    half = nch // 2
    solo = [(c + off, prio(c + off) ^ flip)
            for c in range(half) for off, flip in ((0, 0), (half, 1))]
    solo += [(c, prio(c)) for c in range(2 * half, nch)]

    def kernel_function(q_hbm, k_hbm, v_hbm, o_ref,
                        kb, vb, qb, qf, of, pb, lb, sems, qsem):
        def copy(src, dst, sem_row, head, slot, c):
            return pltpu.make_async_copy(
                src.at[head, pl.ds(c * rows, rows)],
                dst.at[slot, pl.ds(c * rows, rows)],
                sems.at[sem_row, slot])

        def start(u, kslot, vslot):
            for c in range(nch):
                copy(k_hbm, kb, 0, u + 1, kslot, c).start(priority=prio(c))
                copy(v_hbm, vb, 1, u, vslot, c).start(priority=1 - prio(c))

        def start_solo(src, dst, sem_row, head, slot):
            for c, pq in solo:
                copy(src, dst, sem_row, head, slot, c).start(priority=pq)

        def wait(buf, sem_row, slot):
            pltpu.make_async_copy(
                buf.at[slot], buf.at[slot], sems.at[sem_row, slot]).wait()

        def softmax_weights(h, slot, par):
            qh = qf[pl.ds(h * G, G), :].astype(jnp.bfloat16)
            s = jax.lax.dot_general(
                qh, kb[slot], (((1,), (1,)), ((), ())),
                preferred_element_type=jnp.float32) * scale
            m = jnp.max(s, axis=-1, keepdims=True)
            p = jnp.exp(s - m)
            lb[par] = jnp.broadcast_to(jnp.sum(p, axis=-1, keepdims=True), (G, D))
            pb[par] = p.astype(jnp.bfloat16)

        def weighted_sum(h, slot, par):
            o = jnp.dot(pb[par], vb[slot], preferred_element_type=jnp.float32)
            of[pl.ds(h * G, G), :] = o / lb[par]

        q_copy = pltpu.make_async_copy(q_hbm, qb, qsem)
        q_copy.start()
        start_solo(k_hbm, kb, 0, 0, 0)
        for u in range(_INFLIGHT - 1):
            start(u, (u + 1) % _NSLOTS, u % _NSLOTS)
        q_copy.wait()
        qf[...] = qb[...].astype(jnp.float32)
        wait(kb, 0, 0)
        start(_INFLIGHT - 1, _INFLIGHT % _NSLOTS, (_INFLIGHT - 1) % _NSLOTS)
        softmax_weights(0, 0, 0)

        def body(u, carry):
            kslot = jax.lax.rem(u + 1, _NSLOTS)
            vslot = jax.lax.rem(u, _NSLOTS)
            wait(kb, 0, kslot)
            wait(vb, 1, vslot)
            nxt = u + _INFLIGHT

            @pl.when(nxt < N - 1)
            def _():
                start(nxt, jax.lax.rem(nxt + 1, _NSLOTS), jax.lax.rem(nxt, _NSLOTS))

            @pl.when(nxt == N - 1)
            def _():
                start_solo(v_hbm, vb, 1, N - 1, (N - 1) % _NSLOTS)

            par = jax.lax.rem(u, 2)
            weighted_sum(u, vslot, par)
            softmax_weights(u + 1, kslot, 1 - par)
            return carry

        jax.lax.fori_loop(0, N - 1, body, 0)
        wait(vb, 1, (N - 1) % _NSLOTS)
        weighted_sum(N - 1, (N - 1) % _NSLOTS, (N - 1) % 2)
        o_ref[...] = of[...].astype(o_ref.dtype)

    out = pl.pallas_call(
        kernel_function,
        in_specs=[pl.BlockSpec(memory_space=pl.ANY)] * 3,
        out_specs=pl.BlockSpec(memory_space=pltpu.VMEM),
        out_shape=jax.ShapeDtypeStruct((N * G, D), q.dtype),
        scratch_shapes=[
            pltpu.VMEM((_NSLOTS, Sk, D), k.dtype),
            pltpu.VMEM((_NSLOTS, Sk, D), v.dtype),
            pltpu.VMEM((N * G, D), q.dtype),
            pltpu.VMEM((N * G, D), jnp.float32),
            pltpu.VMEM((N * G, D), jnp.float32),
            pltpu.VMEM((2, G, Sk), jnp.bfloat16),
            pltpu.VMEM((2, G, D), jnp.float32),
            pltpu.SemaphoreType.DMA((2, _NSLOTS)),
            pltpu.SemaphoreType.DMA(()),
        ],
        compiler_params=pltpu.CompilerParams(vmem_limit_bytes=64 * 1024 * 1024),
    )(q2, k3, v3)
    return out.reshape(B, Hq, Sq, D)
```
